```python
import os as _os
_os.environ.setdefault("JAX_PLATFORMS", "cpu")
import jax
import jax.numpy as jnp

def _softmax(x, axis=-1):
    return jax.nn.softmax(x, axis=axis)
def _gelu(x):
    return jax.nn.gelu(x, approximate=True)
def _silu(x):
    return jax.nn.silu(x)
def _sigmoid(x):
    return jax.nn.sigmoid(x)
def _layernorm(x, axis=-1, eps=1e-5):
    m = jnp.mean(x, axis=axis, keepdims=True)
    v = jnp.var(x, axis=axis, keepdims=True)
    return (x - m) / jnp.sqrt(v + eps)
def _scatter_add(tgt, idx, src, axis=0):
    return tgt.at[idx].add(src)
def _segment_sum(src, seg, n):
    return jax.ops.segment_sum(src, seg, n)
class _Rng:
    def __init__(self, key):
        self._k = key
    def _next(self):
        self._k, sub = jax.random.split(self._k)
        return sub
    def normal(self, shape):
        return jax.random.normal(self._next(), shape, dtype=jnp.bfloat16)
    def randint(self, lo, hi, shape):
        return jax.random.randint(self._next(), shape, lo, hi, dtype=jnp.int32)
    def uniform(self, shape, lo=0.0, hi=1.0):
        return jax.random.uniform(self._next(), shape, jnp.bfloat16, lo, hi)
    def permutation(self, n):
        return jax.random.permutation(self._next(), n)


kernel_name = 'standalone__sliding_local_fixed_window__prompt'

def setup_inputs():
    _rng = _Rng(jax.random.key(int.from_bytes(__import__("os").urandom(4), "little")))
    _w = (lambda a: (lambda t: t.astype(jnp.bfloat16) if jnp.issubdtype(t.dtype, jnp.floating) else t)(jnp.asarray(a)))
    B, H, S, D = 1, 32, 2048, 128
    return {
        "q": _w((lambda *s: _rng.normal(s) * 0.4)(B, H, S, D)),
        "k": _w((lambda *s: _rng.normal(s) * 0.4)(B, H, S, D)),
        "v": _w((lambda *s: _rng.normal(s) * 0.05)(B, H, S, D)),
    }

def reference(q, k, v):
    B, H, S, D = q.shape
    w = 32
    pos = jnp.arange(S)
    rel = pos[:, None] - pos[None, :]
    mask = (rel >= 0) & (rel < w)
    scores = jnp.einsum("bhqd,bhkd->bhqk", q, k) * (D ** -0.5)
    scores = jnp.where(mask[None, None], scores, (lambda x, dt: x.astype(dt))(jnp.array(-1e9), q.dtype))
    p = _softmax(scores, axis=-1)
    return jnp.einsum("bhqk,bhkd->bhqd", p, v)
```

```python
import functools
import math

import jax
import jax.numpy as jnp
import jax.experimental.pallas as pl
import jax.experimental.pallas.tpu as pltpu

W = 32
KW = 128
TQ = KW - W
NEG = -1e30

T = 256
NG = 2
LA = 3
LW = 12


def _attend(q, k, v, off, c):
    m_rows = q.shape[0]
    s = jax.lax.dot_general(q, k, (((1,), (1,)), ((), ())),
                            preferred_element_type=jnp.float32)
    r = jax.lax.broadcasted_iota(jnp.int32, (m_rows, KW), 0) + off
    j = jax.lax.broadcasted_iota(jnp.int32, (m_rows, KW), 1)
    rel = r - j
    s = jnp.where((rel >= 0) & (rel < W), s, NEG)
    m = jnp.max(s, axis=-1, keepdims=True)
    p = jnp.exp2((s - m) * c)
    l = jnp.sum(p, axis=-1, keepdims=True)
    o = jnp.dot(p.astype(jnp.bfloat16), v, preferred_element_type=jnp.float32)
    return o * pl.reciprocal(l, approx=True)


def _kernel(q_hbm, k_hbm, v_hbm, o_hbm, qb, kb, vb, ob, gsem, isem, *, NH, S, c):
    h = pl.program_id(0)
    pairs = ((q_hbm, qb), (k_hbm, kb), (v_hbm, vb))
    RPH = 3 * (S // T)
    WPH = S // T
    GS = RPH // NG
    NSG = LA + 1
    NW = NH * WPH
    tiles = [(0, KW, 0, 0)] + [(KW + TQ * i, TQ, KW + TQ * i - W, W)
                               for i in range((S - KW) // TQ)]
    rows_per_group = S // NG

    def gsem_at(hh, g):
        gg = hh * NG + g
        if isinstance(gg, int):
            return gsem.at[gg % NSG]
        return gsem.at[jax.lax.rem(gg, NSG)]

    def rcopy(hh, j):
        src, dst = pairs[j % 3]
        r0 = (j // 3) * T
        return pltpu.make_async_copy(src.at[hh, pl.ds(r0, T), :], dst.at[hh, pl.ds(r0, T), :],
                                     gsem_at(hh, j // GS))

    def wcopy(w, sem):
        if isinstance(w, int):
            hh, r0 = w // WPH, (w % WPH) * T
        else:
            hh = w // WPH
            r0 = pl.multiple_of((w % WPH) * T, T)
        return pltpu.make_async_copy(ob.at[hh, pl.ds(r0, T), :], o_hbm.at[hh, pl.ds(r0, T), :], sem)

    def wsem(w):
        return gsem_at(NH, w // GS) if w < LA * GS else isem.at[w % LW]

    @pl.when(h == 0)
    def _():
        for i in range(LA * GS):
            rcopy(i // RPH, i % RPH).start(priority=i % 2)

    t = 0
    for g in range(NG):
        for d in range(GS):
            rcopy(h, g * GS + d).wait()
        hs = h + (g + LA) // NG
        gs = (g + LA) % NG
        for e in range((g + LA) // NG):
            @pl.when(hs == NH + e)
            def _():
                for d in range(GS):
                    w = e * RPH + gs * GS + d
                    wcopy(w, wsem(w)).start(priority=w % 2)
        seg = [tl for tl in tiles if g * rows_per_group < tl[0] + tl[1] <= (g + 1) * rows_per_group]
        for tt, (q0, nq, k0, off) in enumerate(seg):
            for d in range(GS):
                if d * len(seg) // GS == tt:
                    j = gs * GS + d

                    @pl.when(hs < NH)
                    def _():
                        rcopy(hs, j).start(priority=j % 2)
            ob[h, q0:q0 + nq, :] = _attend(qb[h, q0:q0 + nq, :], kb[h, k0:k0 + KW, :],
                                           vb[h, k0:k0 + KW, :], off, c).astype(ob.dtype)
            t += 1
    assert t == len(tiles)

    @pl.when(h == NH - 1)
    def _():
        base = LA * GS
        nstarted = base
        for g in range(LA):
            for d in range(GS):
                w = g * GS + d
                wcopy(w, wsem(w)).wait()
            while (LA - 1 - g) * GS + (nstarted - base) < LW:
                wcopy(nstarted, wsem(nstarted)).start(priority=nstarted % 2)
                nstarted += 1
        assert nstarted - base == LW and (NW - nstarted) % 2 == 0

        def body(i, carry):
            for u in range(2):
                w = nstarted + 2 * i + u
                sem = isem.at[jax.lax.rem(w, LW)]
                wcopy(w - LW, sem).wait()
                wcopy(w, sem).start(priority=(nstarted + u) % 2)
            return carry
        jax.lax.fori_loop(0, (NW - nstarted) // 2, body, 0)
        for w in range(NW - LW, NW):
            wcopy(w, wsem(w)).wait()


@jax.jit
def pallas_standalone__sliding_local_fixed_window__prompt_kernel(q, k, v):
    B, H, S, D = q.shape
    NH = B * H
    c = (D ** -0.5) * math.log2(math.e)
    q3, k3, v3 = [x.reshape(NH, S, D) for x in (q, k, v)]
    spec = pl.BlockSpec(memory_space=pl.ANY)
    o = pl.pallas_call(
        functools.partial(_kernel, NH=NH, S=S, c=c),
        grid=(NH,),
        in_specs=[spec, spec, spec],
        out_specs=spec,
        out_shape=jax.ShapeDtypeStruct((NH, S, D), q.dtype),
        scratch_shapes=[pltpu.VMEM((NH, S, D), q.dtype)] * 4 + [
            pltpu.SemaphoreType.DMA((LA + 1,)), pltpu.SemaphoreType.DMA((LW,))],
        compiler_params=pltpu.CompilerParams(
            dimension_semantics=("arbitrary",),
            disable_bounds_checks=True,
            vmem_limit_bytes=100 * 1024 * 1024),
    )(q3, k3, v3)
    return o.reshape(B, H, S, D)
```

```python
import functools
import math

import jax
import jax.numpy as jnp
import jax.experimental.pallas as pl
import jax.experimental.pallas.tpu as pltpu

W = 32
KW = 128
TQ = KW - W
NEG = -1e30

TR = 128
TW = 256
LA = 4
WR = 8


def _attend(q, k, v, off, c):
    m_rows = q.shape[0]
    s = jax.lax.dot_general(q, k, (((1,), (1,)), ((), ())),
                            preferred_element_type=jnp.float32)
    r = jax.lax.broadcasted_iota(jnp.int32, (m_rows, KW), 0) + off
    j = jax.lax.broadcasted_iota(jnp.int32, (m_rows, KW), 1)
    rel = r - j
    s = jnp.where((rel >= 0) & (rel < W), s, NEG)
    m = jnp.max(s, axis=-1, keepdims=True)
    p = jnp.exp2((s - m) * c)
    l = jnp.sum(p, axis=-1, keepdims=True)
    o = jnp.dot(p.astype(jnp.bfloat16), v, preferred_element_type=jnp.float32)
    return o * pl.reciprocal(l, approx=True)


def _kernel(q_hbm, k_hbm, v_hbm, o_hbm, qb, kb, vb, ob, rsem, wsem, *, NH, S, c):
    half = NH // 2
    nc = S // TR
    wph = S // TW
    pairs = ((q_hbm, qb), (k_hbm, kb), (v_hbm, vb))

    s = pl.program_id(0)
    h = s // 2 + (s % 2) * half

    def rcopy(hh, a, r0):
        src, dst = pairs[a]
        return pltpu.make_async_copy(src.at[hh, pl.ds(r0, TR), :], dst.at[hh, pl.ds(r0, TR), :],
                                     rsem.at[hh])

    def issue_reads(slot):
        p = slot // 2
        base = (slot % 2) * (S // 2)
        if not isinstance(base, int):
            base = pl.multiple_of(base, S // 2)
        i = 0
        for ch in range(nc // 2):
            for hh in (p, p + half):
                for a in range(3):
                    rcopy(hh, a, base + ch * TR).start(priority=i % 2)
                    i += 1

    worder = [(st // 2 + (st % 2) * half, ch)
              for blk in range(NH // WR) for ch in range(wph)
              for st in range(blk * WR, (blk + 1) * WR)]
    per_block = WR * wph

    def wcopy(i):
        hh, ch = worder[i]
        return pltpu.make_async_copy(ob.at[hh, pl.ds(ch * TW, TW), :],
                                     o_hbm.at[hh, pl.ds(ch * TW, TW), :], wsem.at[0])

    def issue_writes(lo, hi):
        for i in range(lo, hi):
            wcopy(i).start(priority=i % 2)

    @pl.when(s == 0)
    def _():
        for slot in range(LA):
            issue_reads(slot)

    for ch in range(nc):
        for a in range(3):
            rcopy(h, a, ch * TR).wait()

    @pl.when(s + LA < NH)
    def _():
        issue_reads(s + LA)

    @pl.when(s == NH - 3)
    def _():
        issue_writes(0, per_block)

    @pl.when(s == NH - 2)
    def _():
        issue_writes(per_block, len(worder) - per_block)

    ob[h, 0:KW, :] = _attend(qb[h, 0:KW, :], kb[h, 0:KW, :], vb[h, 0:KW, :], 0, c).astype(ob.dtype)
    for t in range((S - KW) // TQ):
        q0 = KW + TQ * t
        k0 = q0 - W
        ob[h, q0:q0 + TQ, :] = _attend(qb[h, q0:q0 + TQ, :], kb[h, k0:k0 + KW, :],
                                       vb[h, k0:k0 + KW, :], W, c).astype(ob.dtype)

    @pl.when(s == NH - 1)
    def _():
        issue_writes(len(worder) - per_block, len(worder))
        for i in range(len(worder)):
            wcopy(i).wait()


@jax.jit
def pallas_standalone__sliding_local_fixed_window__prompt_kernel(q, k, v):
    B, H, S, D = q.shape
    NH = B * H
    assert D == KW and (S - KW) % TQ == 0 and S % (2 * TR) == 0 and S % TW == 0
    assert NH % WR == 0 and NH >= 2 * WR and WR >= 4 and LA % 2 == 0
    c = (D ** -0.5) * math.log2(math.e)
    q3, k3, v3 = [x.reshape(NH, S, D) for x in (q, k, v)]
    spec = pl.BlockSpec(memory_space=pl.ANY)
    o = pl.pallas_call(
        functools.partial(_kernel, NH=NH, S=S, c=c),
        grid=(NH,),
        in_specs=[spec, spec, spec],
        out_specs=spec,
        out_shape=jax.ShapeDtypeStruct((NH, S, D), q.dtype),
        scratch_shapes=[pltpu.VMEM((NH, S, D), q.dtype)] * 4 + [
            pltpu.SemaphoreType.DMA((NH,)), pltpu.SemaphoreType.DMA((1,))],
        compiler_params=pltpu.CompilerParams(
            dimension_semantics=("arbitrary",),
            disable_bounds_checks=True,
            vmem_limit_bytes=100 * 1024 * 1024),
    )(q3, k3, v3)
    return o.reshape(B, H, S, D)
```

```python
import functools
import math

import jax
import jax.numpy as jnp
import jax.experimental.pallas as pl
import jax.experimental.pallas.tpu as pltpu

W = 32
KW = 128
TQ = KW - W
NEG = -1e30

TR = 128
TW = 128
LA = 4
NSEM = 8
WR = 8


def _attend(q, k, v, off, c):
    m_rows = q.shape[0]
    s = jax.lax.dot_general(q, k, (((1,), (1,)), ((), ())),
                            preferred_element_type=jnp.float32)
    r = jax.lax.broadcasted_iota(jnp.int32, (m_rows, KW), 0) + off
    j = jax.lax.broadcasted_iota(jnp.int32, (m_rows, KW), 1)
    rel = r - j
    s = jnp.where((rel >= 0) & (rel < W), s, NEG)
    m = jnp.max(s, axis=-1, keepdims=True)
    p = jnp.exp2((s - m) * c)
    l = jnp.sum(p, axis=-1, keepdims=True)
    o = jnp.dot(p.astype(jnp.bfloat16), v, preferred_element_type=jnp.float32)
    return o / l


def _kernel(q_hbm, k_hbm, v_hbm, o_hbm, qb, kb, vb, ob, rsem, wsem, *, NH, S, c):
    half = NH // 2
    nc = S // TR
    wph = S // TW
    pairs = ((q_hbm, qb), (k_hbm, kb), (v_hbm, vb))

    s = pl.program_id(0)
    h = s // 2 + (s % 2) * half

    def rcopy(hh, a, r0, step):
        src, dst = pairs[a]
        return pltpu.make_async_copy(src.at[hh, pl.ds(r0, TR), :], dst.at[hh, pl.ds(r0, TR), :],
                                     rsem.at[step % NSEM])

    def issue_reads(slot):
        p = slot // 2
        base = (slot % 2) * (S // 2)
        if not isinstance(base, int):
            base = pl.multiple_of(base, S // 2)
        i = 0
        for ch in range(nc // 2):
            for a in range(3):
                for u in range(2):
                    rcopy(p + u * half, a, base + ch * TR, 2 * p + u).start(priority=i % 2)
                    i += 1

    worder = [(st // 2 + (st % 2) * half, ch)
              for blk in range(NH // WR) for ch in range(wph)
              for st in range(blk * WR, (blk + 1) * WR)]
    per_block = WR * wph

    def wcopy(i):
        hh, ch = worder[i]
        return pltpu.make_async_copy(ob.at[hh, pl.ds(ch * TW, TW), :],
                                     o_hbm.at[hh, pl.ds(ch * TW, TW), :], wsem.at[0])

    def issue_writes(lo, hi):
        for i in range(lo, hi):
            wcopy(i).start(priority=i % 2)

    @pl.when(s == 0)
    def _():
        for slot in range(LA):
            issue_reads(slot)

    for ch in range(nc):
        for a in range(3):
            rcopy(h, a, ch * TR, s).wait()

    @pl.when(s + LA < NH)
    def _():
        issue_reads(s + LA)

    @pl.when(s == NH - 3)
    def _():
        issue_writes(0, per_block)

    @pl.when(s == NH - 2)
    def _():
        issue_writes(per_block, len(worder) - per_block)

    ob[h, 0:KW, :] = _attend(qb[h, 0:KW, :], kb[h, 0:KW, :], vb[h, 0:KW, :], 0, c).astype(ob.dtype)
    for t in range((S - KW) // TQ):
        q0 = KW + TQ * t
        k0 = q0 - W
        ob[h, q0:q0 + TQ, :] = _attend(qb[h, q0:q0 + TQ, :], kb[h, k0:k0 + KW, :],
                                       vb[h, k0:k0 + KW, :], W, c).astype(ob.dtype)

    @pl.when(s == NH - 1)
    def _():
        issue_writes(len(worder) - per_block, len(worder))
        for i in range(len(worder)):
            wcopy(i).wait()


@jax.jit
def pallas_standalone__sliding_local_fixed_window__prompt_kernel(q, k, v):
    B, H, S, D = q.shape
    NH = B * H
    assert D == KW and (S - KW) % TQ == 0 and S % (2 * TR) == 0 and S % TW == 0
    assert NH % WR == 0 and NH >= 2 * WR and WR >= 4 and LA % 2 == 0 and NSEM >= LA + 2
    c = (D ** -0.5) * math.log2(math.e)
    q3, k3, v3 = [x.reshape(NH, S, D) for x in (q, k, v)]
    spec = pl.BlockSpec(memory_space=pl.ANY)
    o = pl.pallas_call(
        functools.partial(_kernel, NH=NH, S=S, c=c),
        grid=(NH,),
        in_specs=[spec, spec, spec],
        out_specs=spec,
        out_shape=jax.ShapeDtypeStruct((NH, S, D), q.dtype),
        scratch_shapes=[pltpu.VMEM((NH, S, D), q.dtype)] * 4 + [
            pltpu.SemaphoreType.DMA((NSEM,)), pltpu.SemaphoreType.DMA((1,))],
        compiler_params=pltpu.CompilerParams(
            dimension_semantics=("arbitrary",),
            disable_bounds_checks=True,
            disable_semaphore_checks=True,
            vmem_limit_bytes=100 * 1024 * 1024),
    )(q3, k3, v3)
    return o.reshape(B, H, S, D)
```
